```python
import jax
import jax.numpy as jnp

def _softmax(x, axis=-1):
    return jax.nn.softmax(x, axis=axis)
def _gelu(x):
    return jax.nn.gelu(x, approximate=True)
def _silu(x):
    return jax.nn.silu(x)
def _sigmoid(x):
    return jax.nn.sigmoid(x)
def _layernorm(x, axis=-1, eps=1e-5):
    m = jnp.mean(x, axis=axis, keepdims=True)
    v = jnp.var(x, axis=axis, keepdims=True)
    return (x - m) / jnp.sqrt(v + eps)
def _scatter_add(tgt, idx, src, axis=0):
    return tgt.at[idx].add(src)
def _segment_sum(src, seg, n):
    return jax.ops.segment_sum(src, seg, n)
class _Rng:
    def __init__(self, key):
        self._k = key
    def _next(self):
        self._k, sub = jax.random.split(self._k)
        return sub
    def normal(self, shape):
        return jax.random.normal(self._next(), shape, dtype=jnp.bfloat16)
    def randint(self, lo, hi, shape):
        return jax.random.randint(self._next(), shape, lo, hi, dtype=jnp.int32)
    def uniform(self, shape, lo=0.0, hi=1.0):
        return jax.random.uniform(self._next(), shape, jnp.bfloat16, lo, hi)
    def permutation(self, n):
        return jax.random.permutation(self._next(), n)


kernel_name = 'interleave_layers__softmax_full_mha__ssm_conv_h3__prompt'

def setup_inputs():
    _rng = _Rng(jax.random.key(int.from_bytes(__import__("os").urandom(4), "little")))
    _w = (lambda a: (lambda t: t.astype(jnp.bfloat16) if jnp.issubdtype(t.dtype, jnp.floating) else t)(jnp.asarray(a)))
    def _A_setup():
        B, S, D = 1, 2048, 1024
        return {
            "x": _w((lambda *s: _rng.normal(s) * 0.05)(B, S, D)),
            "wqkv": _w((lambda *s: _rng.normal(s) * 0.05)(D, 3 * D)),
            "wo": _w((lambda *s: _rng.normal(s) * 0.05)(D, D)),
        }
    _A_in = _A_setup()

    def _B_setup():
        B, S, D = 1, 2048, 1024
        ks = 4
        return {
            "q": _w((lambda *s: _rng.normal(s) * 0.05)(B, S, D)),
            "k": _w((lambda *s: _rng.normal(s) * 0.05)(B, S, D)),
            "v": _w((lambda *s: _rng.normal(s) * 0.05)(B, S, D)),
            "shift_k": _w((lambda *s: _rng.normal(s) * 0.05)(D, ks) * 0.5),
            "ssm_k": _w((lambda *s: _rng.normal(s) * 0.05)(D, S) * (1.0 / S ** 0.5)),
            "ssm_D": _w((lambda *s: _rng.normal(s) * 0.05)(D)),
        }
    _B_in = _B_setup()

    return {
        "A_x": _A_in["x"],
        "A_wqkv": _A_in["wqkv"],
        "A_wo": _A_in["wo"],
        "B_q": _B_in["q"],
        "B_k": _B_in["k"],
        "B_v": _B_in["v"],
        "B_shift_k": _B_in["shift_k"],
        "B_ssm_k": _B_in["ssm_k"],
        "B_ssm_D": _B_in["ssm_D"],
    }

def reference(A_x, A_wqkv, A_wo, B_q, B_k, B_v, B_shift_k, B_ssm_k, B_ssm_D):
    def _A_ref(x, wqkv, wo):
        B, S, D = x.shape
        H = 32; Dh = D // H
        qkv = (lambda x, *d: x.transpose(*d))((x @ wqkv).reshape(B, S, 3, H, Dh), 2, 0, 3, 1, 4)
        q, k, v = qkv[0], qkv[1], qkv[2]
        scale = Dh ** -0.5
        scores = jnp.einsum("bhqd,bhkd->bhqk", q, k) * scale
        p = _softmax(scores, axis=-1)
        o = jnp.einsum("bhqk,bhkd->bhqd", p, v)
        return (lambda x, *d: x.transpose(*d))(o, 0, 2, 1, 3).reshape(B, S, D) @ wo

    def _B_ref(q, k, v, shift_k, ssm_k, ssm_D):
        B, S, D = q.shape
        ks = shift_k.shape[-1]
        k_pad = jnp.pad(k, ((0, 0), (ks - 1, 0), (0, 0)))
        k_shift = jnp.zeros_like(k)
        for t in range(ks):
            k_shift = k_shift + k_pad[:, t:t + S, :] * shift_k[:, ks - 1 - t][None, None, :]
        kv = k_shift * v
        L = 2 * S
        kv_pad = jnp.pad(kv, ((0, 0), (0, S), (0, 0)))
        kf_pad = jnp.pad(ssm_k, ((0, 0), (0, S)))
        kv_f = (lambda x, axes=(-2,-1): jnp.fft.rfft2(x.astype(jnp.float32), axes=axes))(kv_pad[:, None, :, :], axes=(1, 2))
        kf_f = (lambda x, axes=(-2,-1): jnp.fft.rfft2(x.astype(jnp.float32), axes=axes))(kf_pad[:, None, :], axes=(1, 2))
        kf_f = (lambda x, *d: x.transpose(*d))(kf_f, 1, 2, 0)
        y_f = kv_f * kf_f[None, :, :, :]
        y = (lambda x, s, axes=(-2,-1): jnp.fft.irfft2(x, s=s, axes=axes).astype(jnp.bfloat16))(y_f, (1, L), axes=(1, 2))[:, 0, :S, :]
        y = y + kv * ssm_D[None, None, :]
        return q * y

    x = A_x
    x = x + _A_ref(_layernorm(x, axis=-1), A_wqkv, A_wo)
    x = x + _B_ref(_layernorm(x, axis=-1), B_k, B_v, B_shift_k, B_ssm_k, B_ssm_D)
    x = x + _A_ref(_layernorm(x, axis=-1), A_wqkv, A_wo)
    x = x + _B_ref(_layernorm(x, axis=-1), B_k, B_v, B_shift_k, B_ssm_k, B_ssm_D)
    return x
```

```python
import jax
import jax.numpy as jnp
import numpy as np
from jax import lax
import jax.experimental.pallas as pl
import jax.experimental.pallas.tpu as pltpu

S, D, H, DH = 2048, 1024, 32, 32
TQ, KC, RB, C = 512, 128, 256, 128
NT = (((1,), (1,)), ((), ()))
F32, BF16 = jnp.float32, jnp.bfloat16


def _dft_mats():
    k = np.arange(C)[:, None] + 0.5
    n = np.arange(C)[None, :]
    a = 2 * np.pi * k * n / (2 * C)
    fwd = np.concatenate([np.cos(a), -np.sin(a)], 0)
    inv = np.concatenate([np.cos(a).T, -np.sin(a).T], 1) / C
    return np.concatenate([fwd, inv.T], 0).astype(np.float32)


def _ln(x):
    m = jnp.mean(x, axis=-1, keepdims=True)
    c = x - m
    v = jnp.mean(c * c, axis=-1, keepdims=True)
    return c * lax.rsqrt(v + 1e-5)


def _kernel(f_ref, sk_ref, sd_ref, x_hbm, wqkv_hbm, wo_hbm, bk_hbm, bv_hbm, ssm_hbm, o_ref,
            xin, wqkv, wo, bk, bv, ssm, x, y, q_ref, k_ref, vt_ref, ot_ref, sa, sb, kp, xf, hf, sem):
    cps = [pltpu.make_async_copy(a, b, sem.at[i]) for i, (a, b) in enumerate(
        [(bk_hbm, bk), (bv_hbm, bv), (ssm_hbm, ssm), (x_hbm, xin), (wqkv_hbm, wqkv), (wo_hbm, wo)])]
    for cp in cps:
        cp.start()
    for cp in cps[:3]:
        cp.wait()

    with jax.named_scope("conv"):
        fwd = f_ref[0:2 * C, :].astype(BF16)
        inv = f_ref[2 * C:4 * C, :].T.astype(BF16)
        sgn = (1 - 2 * (lax.broadcasted_iota(jnp.int32, (C, 128), 0) & 1)).astype(F32)
        NCH = S // C
        kp[0:8, :] = jnp.zeros((8, 128), F32)

        def conv_body(d, carry):
            dl = pl.ds(pl.multiple_of(d * 128, 128), 128)
            kp[8:, :] = bk[:, dl].astype(F32)
            w = sk_ref[:, dl].astype(F32)
            dd = sd_ref[:, dl].astype(F32)
            prev = None
            for j in range(NCH):
                ks = kp[8 + j * C:8 + (j + 1) * C, :] * w[0:1]
                for t in range(1, 4):
                    ks = ks + kp[8 + j * C - t:8 + (j + 1) * C - t, :] * w[t:t + 1]
                kv = ks * bv[j * C:(j + 1) * C, dl].astype(F32)
                y[j * C:(j + 1) * C, dl] = kv * dd
                xf[j] = jnp.dot(fwd, kv.astype(BF16), preferred_element_type=F32)
                kf = lax.dot_general(fwd, ssm[dl, j * C:(j + 1) * C], NT, preferred_element_type=F32)
                if prev is None:
                    hf[j] = kf
                else:
                    hf[j, 0:C] = kf[:C] - sgn * prev[C:]
                    hf[j, C:] = kf[C:] + sgn * prev[:C]
                prev = kf
            for i in range(NCH):
                zr = zi = None
                for j in range(i + 1):
                    ar, ai = xf[j, 0:C], xf[j, C:]
                    br, bi = hf[i - j, 0:C], hf[i - j, C:]
                    pr, pi = ar * br - ai * bi, ar * bi + ai * br
                    zr = pr if zr is None else zr + pr
                    zi = pi if zi is None else zi + pi
                z = jnp.concatenate([zr, zi], 0).astype(BF16)
                y[i * C:(i + 1) * C, dl] += jnp.dot(inv, z, preferred_element_type=F32)
            return carry
        lax.fori_loop(0, D // 128, conv_body, 0)

    for cp in cps[3:]:
        cp.wait()
    x[...] = xin[...].astype(F32)

    lane = lax.broadcasted_iota(jnp.int32, (TQ, 128), 1) // DH
    nq = S // TQ
    nb = H * nq
    nc = S // KC

    def attn_step(i, m_cur, s_cur, s_nxt, do_pv=True):
        n = jnp.minimum(i + 1, nb - 1)
        hn = n // nq
        g = pl.ds(pl.multiple_of((hn // 4) * 128, 128), 128)
        q4 = q_ref[pl.ds(pl.multiple_of((n % nq) * TQ, TQ), TQ), g].astype(F32)
        qm = jnp.where(lane == hn % 4, q4, 0.0).astype(BF16)
        mp = jnp.full((8, TQ), -jnp.inf, F32)
        if do_pv:
            hs = pl.ds(pl.multiple_of((i // nq) * DH, DH), DH)
            lp = jnp.zeros((8, TQ), F32)
            acc = jnp.zeros((DH, TQ), F32)
        for c in range(nc):
            r = slice(c * KC, (c + 1) * KC)
            st = lax.dot_general(k_ref[r, g], qm, NT, preferred_element_type=F32)
            s_nxt[r, :] = st
            mp = jnp.maximum(mp, jnp.max(st.reshape(KC // 8, 8, TQ), axis=0))
            if do_pv:
                p = jnp.exp2(s_cur[r, :] - m_cur)
                lp = lp + jnp.sum(p.reshape(KC // 8, 8, TQ), axis=0)
                acc = acc + jnp.dot(vt_ref[hs, r], p.astype(BF16), preferred_element_type=F32)
        if do_pv:
            l = jnp.sum(lp, axis=0, keepdims=True)
            ot_ref[hs, pl.ds(pl.multiple_of((i % nq) * TQ, TQ), TQ)] = (acc / l).astype(BF16)
        return jnp.max(mp, axis=0, keepdims=True)

    def layer(_, carry):
        with jax.named_scope("qkv"):
            def qkv_body(b, c):
                for u in range(2):
                    r = pl.ds(pl.multiple_of((b * 2 + u) * RB, RB), RB)
                    xn = _ln(x[r, :]).astype(BF16)
                    qv = jnp.dot(xn, wqkv[:, 0:D], preferred_element_type=F32)
                    q_ref[r, :] = (qv * float(DH ** -0.5 * np.log2(np.e))).astype(BF16)
                    k_ref[r, :] = jnp.dot(xn, wqkv[:, D:2 * D], preferred_element_type=F32).astype(BF16)
                    vt_ref[:, r] = jnp.dot(xn, wqkv[:, 2 * D:], preferred_element_type=F32).T.astype(BF16)
                return c
            lax.fori_loop(0, S // RB // 2, qkv_body, 0)
        with jax.named_scope("attn"):
            m0 = attn_step(-1, None, sb, sa, do_pv=False)

            def abody(j, m):
                m = attn_step(2 * j, m, sa, sb)
                return attn_step(2 * j + 1, m, sb, sa)
            lax.fori_loop(0, nb // 2, abody, m0)
        with jax.named_scope("outp"):
            def out_body(b, c):
                for u in range(2):
                    r = pl.ds(pl.multiple_of((b * 2 + u) * RB, RB), RB)
                    o = ot_ref[:, r].astype(F32).T.astype(BF16)
                    xr = x[r, :] + jnp.dot(o, wo[...], preferred_element_type=F32)
                    xr = xr + _ln(xr) * y[r, :]
                    x[r, :] = xr
                    o_ref[r, :] = xr.astype(BF16)
                return c
            lax.fori_loop(0, S // RB // 2, out_body, 0)
        return carry
    lax.fori_loop(0, 2, layer, 0)


@jax.jit
def pallas_interleave_layers__softmax_full_mha__ssm_conv_h3__prompt_kernel(
    A_x: jax.Array,
    A_wqkv: jax.Array,
    A_wo: jax.Array,
    B_q: jax.Array,
    B_k: jax.Array,
    B_v: jax.Array,
    B_shift_k: jax.Array,
    B_ssm_k: jax.Array,
    B_ssm_D: jax.Array,
):
    vm = pltpu.VMEM
    anys = pl.BlockSpec(memory_space=pl.ANY)
    out = pl.pallas_call(
        _kernel,
        in_specs=[pl.BlockSpec(memory_space=pltpu.VMEM)] * 3 + [anys] * 6,
        out_specs=pl.BlockSpec(memory_space=pltpu.VMEM),
        out_shape=jax.ShapeDtypeStruct((S, D), BF16),
        scratch_shapes=[
            vm((S, D), BF16), vm((D, 3 * D), BF16), vm((D, D), BF16),
            vm((S, D), BF16), vm((S, D), BF16), vm((D, S), BF16),
            vm((S, D), F32), vm((S, D), F32),
            vm((S, D), BF16), vm((S, D), BF16), vm((D, S), BF16), vm((D, S), BF16),
            vm((S, TQ), F32), vm((S, TQ), F32),
            vm((S + 8, 128), F32), vm((S // C, 2 * C, 128), F32), vm((S // C, 2 * C, 128), F32),
            pltpu.SemaphoreType.DMA((6,)),
        ],
        compiler_params=pltpu.CompilerParams(vmem_limit_bytes=110 * 2 ** 20),
    )(_dft_mats(), B_shift_k.T, B_ssm_D.reshape(1, D), A_x.reshape(S, D), A_wqkv, A_wo,
      B_k.reshape(S, D), B_v.reshape(S, D), B_ssm_k)
    return out.reshape(1, S, D)
```

```python
import jax
import jax.numpy as jnp
import numpy as np
from jax import lax
import jax.experimental.pallas as pl
import jax.experimental.pallas.tpu as pltpu

S, D, H, DH = 2048, 1024, 32, 32
TQ, KC, RB, C = 512, 128, 256, 128
NT = (((1,), (1,)), ((), ()))
F32, BF16 = jnp.float32, jnp.bfloat16


def _dft_mats():
    k = np.arange(C)[:, None] + 0.5
    n = np.arange(C)[None, :]
    a = 2 * np.pi * k * n / (2 * C)
    fwd = np.concatenate([np.cos(a), -np.sin(a)], 0)
    inv = np.concatenate([np.cos(a).T, -np.sin(a).T], 1) / C
    return np.concatenate([fwd, inv.T], 0).astype(np.float32)


def _ln(x):
    m = jnp.mean(x, axis=-1, keepdims=True)
    c = x - m
    v = jnp.mean(c * c, axis=-1, keepdims=True)
    return c * lax.rsqrt(v + 1e-5)


def _kernel(f_ref, sk_ref, sd_ref, x_hbm, wqkv_hbm, wo_hbm, bk_hbm, bv_hbm, ssm_hbm, o_ref,
            xin, wqkv, wo, bk, bv, ssm, x, y, q_ref, k_ref, vt_ref, ot_ref, sa, sb, kp, xf, hf, sem, csem):
    def conv_cps(d):
        dl = pl.ds(pl.multiple_of(d * 128, 128), 128)
        return [pltpu.make_async_copy(bk_hbm.at[:, dl], bk.at[:, dl], csem.at[0, d]),
                pltpu.make_async_copy(bv_hbm.at[:, dl], bv.at[:, dl], csem.at[1, d]),
                pltpu.make_async_copy(ssm_hbm.at[dl, :], ssm.at[dl, :], csem.at[2, d])]
    for d in range(D // 128):
        for cp in conv_cps(d):
            cp.start()
    cps = [pltpu.make_async_copy(a, b, sem.at[i]) for i, (a, b) in enumerate(
        [(x_hbm, xin), (wqkv_hbm, wqkv), (wo_hbm, wo)])]
    for cp in cps:
        cp.start()

    with jax.named_scope("conv"):
        fwd = f_ref[0:2 * C, :].astype(BF16)
        inv = f_ref[2 * C:4 * C, :].T.astype(BF16)
        sgn = (1 - 2 * (lax.broadcasted_iota(jnp.int32, (C, 128), 0) & 1)).astype(F32)
        NCH = S // C
        kp[0:8, :] = jnp.zeros((8, 128), F32)

        def conv_body(d, carry):
            dl = pl.ds(pl.multiple_of(d * 128, 128), 128)
            for cp in conv_cps(d):
                cp.wait()
            kp[8:, :] = bk[:, dl].astype(F32)
            w = sk_ref[:, dl].astype(F32)
            dd = sd_ref[:, dl].astype(F32)
            prev = None
            for j in range(NCH):
                ks = kp[8 + j * C:8 + (j + 1) * C, :] * w[0:1]
                for t in range(1, 4):
                    ks = ks + kp[8 + j * C - t:8 + (j + 1) * C - t, :] * w[t:t + 1]
                kv = ks * bv[j * C:(j + 1) * C, dl].astype(F32)
                y[j * C:(j + 1) * C, dl] = kv * dd
                xf[j] = jnp.dot(fwd, kv.astype(BF16), preferred_element_type=F32)
                kf = lax.dot_general(fwd, ssm[dl, j * C:(j + 1) * C], NT, preferred_element_type=F32)
                if prev is None:
                    hf[j] = kf
                else:
                    hf[j, 0:C] = kf[:C] - sgn * prev[C:]
                    hf[j, C:] = kf[C:] + sgn * prev[:C]
                prev = kf
            for i in range(NCH):
                zr = zi = None
                for j in range(i + 1):
                    ar, ai = xf[j, 0:C], xf[j, C:]
                    br, bi = hf[i - j, 0:C], hf[i - j, C:]
                    pr, pi = ar * br - ai * bi, ar * bi + ai * br
                    zr = pr if zr is None else zr + pr
                    zi = pi if zi is None else zi + pi
                z = jnp.concatenate([zr, zi], 0).astype(BF16)
                y[i * C:(i + 1) * C, dl] += jnp.dot(inv, z, preferred_element_type=F32)
            return carry
        lax.fori_loop(0, D // 128, conv_body, 0)

    for cp in cps:
        cp.wait()
    x[...] = xin[...].astype(F32)

    lane = lax.broadcasted_iota(jnp.int32, (TQ, 128), 1) // DH
    nq = S // TQ
    nb = H * nq
    nc = S // KC

    def attn_step(i, m_cur, s_cur, s_nxt, do_pv=True):
        n = jnp.minimum(i + 1, nb - 1)
        hn = n // nq
        g = pl.ds(pl.multiple_of((hn // 4) * 128, 128), 128)
        q4 = q_ref[pl.ds(pl.multiple_of((n % nq) * TQ, TQ), TQ), g].astype(F32)
        qm = jnp.where(lane == hn % 4, q4, 0.0).astype(BF16)
        mp = jnp.full((8, TQ), -jnp.inf, F32)
        if do_pv:
            hs = pl.ds(pl.multiple_of((i // nq) * DH, DH), DH)
            lp = jnp.zeros((8, TQ), F32)
            acc = jnp.zeros((DH, TQ), F32)
        for c in range(nc):
            r = slice(c * KC, (c + 1) * KC)
            st = lax.dot_general(k_ref[r, g], qm, NT, preferred_element_type=F32)
            s_nxt[r, :] = st
            mp = jnp.maximum(mp, jnp.max(st.reshape(KC // 8, 8, TQ), axis=0))
            if do_pv:
                p = jnp.exp2(s_cur[r, :] - m_cur)
                lp = lp + jnp.sum(p.reshape(KC // 8, 8, TQ), axis=0)
                acc = acc + jnp.dot(vt_ref[hs, r], p.astype(BF16), preferred_element_type=F32)
        if do_pv:
            l = jnp.sum(lp, axis=0, keepdims=True)
            ot_ref[hs, pl.ds(pl.multiple_of((i % nq) * TQ, TQ), TQ)] = (acc / l).astype(BF16)
        return jnp.max(mp, axis=0, keepdims=True)

    def layer(_, carry):
        with jax.named_scope("qkv"):
            def qkv_body(b, c):
                for u in range(2):
                    r = pl.ds(pl.multiple_of((b * 2 + u) * RB, RB), RB)
                    xn = _ln(x[r, :]).astype(BF16)
                    qv = jnp.dot(xn, wqkv[:, 0:D], preferred_element_type=F32)
                    q_ref[r, :] = (qv * float(DH ** -0.5 * np.log2(np.e))).astype(BF16)
                    k_ref[r, :] = jnp.dot(xn, wqkv[:, D:2 * D], preferred_element_type=F32).astype(BF16)
                    vt_ref[:, r] = jnp.dot(xn, wqkv[:, 2 * D:], preferred_element_type=F32).T.astype(BF16)
                return c
            lax.fori_loop(0, S // RB // 2, qkv_body, 0)
        with jax.named_scope("attn"):
            m0 = attn_step(-1, None, sb, sa, do_pv=False)

            def abody(j, m):
                m = attn_step(2 * j, m, sa, sb)
                return attn_step(2 * j + 1, m, sb, sa)
            lax.fori_loop(0, nb // 2, abody, m0)
        with jax.named_scope("outp"):
            def out_body(b, c):
                for u in range(2):
                    r = pl.ds(pl.multiple_of((b * 2 + u) * RB, RB), RB)
                    o = ot_ref[:, r].astype(F32).T.astype(BF16)
                    xr = x[r, :] + jnp.dot(o, wo[...], preferred_element_type=F32)
                    xr = xr + _ln(xr) * y[r, :]
                    x[r, :] = xr
                    o_ref[r, :] = xr.astype(BF16)
                return c
            lax.fori_loop(0, S // RB // 2, out_body, 0)
        return carry
    lax.fori_loop(0, 2, layer, 0)


@jax.jit
def pallas_interleave_layers__softmax_full_mha__ssm_conv_h3__prompt_kernel(
    A_x: jax.Array,
    A_wqkv: jax.Array,
    A_wo: jax.Array,
    B_q: jax.Array,
    B_k: jax.Array,
    B_v: jax.Array,
    B_shift_k: jax.Array,
    B_ssm_k: jax.Array,
    B_ssm_D: jax.Array,
):
    vm = pltpu.VMEM
    anys = pl.BlockSpec(memory_space=pl.ANY)
    out = pl.pallas_call(
        _kernel,
        in_specs=[pl.BlockSpec(memory_space=pltpu.VMEM)] * 3 + [anys] * 6,
        out_specs=pl.BlockSpec(memory_space=pltpu.VMEM),
        out_shape=jax.ShapeDtypeStruct((S, D), BF16),
        scratch_shapes=[
            vm((S, D), BF16), vm((D, 3 * D), BF16), vm((D, D), BF16),
            vm((S, D), BF16), vm((S, D), BF16), vm((D, S), BF16),
            vm((S, D), F32), vm((S, D), F32),
            vm((S, D), BF16), vm((S, D), BF16), vm((D, S), BF16), vm((D, S), BF16),
            vm((S, TQ), F32), vm((S, TQ), F32),
            vm((S + 8, 128), F32), vm((S // C, 2 * C, 128), F32), vm((S // C, 2 * C, 128), F32),
            pltpu.SemaphoreType.DMA((3,)), pltpu.SemaphoreType.DMA((3, D // 128)),
        ],
        compiler_params=pltpu.CompilerParams(vmem_limit_bytes=110 * 2 ** 20),
    )(_dft_mats(), B_shift_k.T, B_ssm_D.reshape(1, D), A_x.reshape(S, D), A_wqkv, A_wo,
      B_k.reshape(S, D), B_v.reshape(S, D), B_ssm_k)
    return out.reshape(1, S, D)
```
